```python
import os as _os
_os.environ.setdefault("JAX_PLATFORMS", "cpu")
import jax
import jax.numpy as jnp

def _softmax(x, axis=-1):
    return jax.nn.softmax(x, axis=axis)
def _gelu(x):
    return jax.nn.gelu(x, approximate=True)
def _silu(x):
    return jax.nn.silu(x)
def _sigmoid(x):
    return jax.nn.sigmoid(x)
def _layernorm(x, axis=-1, eps=1e-5):
    m = jnp.mean(x, axis=axis, keepdims=True)
    v = jnp.var(x, axis=axis, keepdims=True)
    return (x - m) / jnp.sqrt(v + eps)
def _scatter_add(tgt, idx, src, axis=0):
    return tgt.at[idx].add(src)
def _segment_sum(src, seg, n):
    return jax.ops.segment_sum(src, seg, n)
class _Rng:
    def __init__(self, key):
        self._k = key
    def _next(self):
        self._k, sub = jax.random.split(self._k)
        return sub
    def normal(self, shape):
        return jax.random.normal(self._next(), shape, dtype=jnp.bfloat16)
    def randint(self, lo, hi, shape):
        return jax.random.randint(self._next(), shape, lo, hi, dtype=jnp.int32)
    def uniform(self, shape, lo=0.0, hi=1.0):
        return jax.random.uniform(self._next(), shape, jnp.bfloat16, lo, hi)
    def permutation(self, n):
        return jax.random.permutation(self._next(), n)


kernel_name = 'sequential_preLN__linear_kernel_hedgehog__geglu_ffn__prompt'

def setup_inputs():
    _rng = _Rng(jax.random.key(int.from_bytes(__import__("os").urandom(4), "little")))
    _w = (lambda a: (lambda t: t.astype(jnp.bfloat16) if jnp.issubdtype(t.dtype, jnp.floating) else t)(jnp.asarray(a)))
    def _A_setup():
        B, S, D, H = 1, 2048, 640, 32
        Dh = D // H
        return {
            "x": _w((lambda *s: _rng.normal(s) * 0.05)(B, S, D)),
            "wqkv": _w((lambda *s: _rng.normal(s) * 0.2)(D, 3 * D)),
            "w_phi": _w((lambda *s: _rng.normal(s) * 0.2)(H, Dh, Dh) * (Dh ** -0.5)),
            "wo": _w((lambda *s: _rng.normal(s) * 0.05)(D, D)),
        }
    _A_in = _A_setup()

    def _B_setup():
        B, S, D, F = 1, 2048, 640, 1536
        return {
            "x": _w((lambda *s: _rng.normal(s) * 0.05)(B, S, D)),
            "w_gate": _w((lambda *s: _rng.normal(s) * 0.05)(D, F)),
            "w_up": _w((lambda *s: _rng.normal(s) * 0.05)(D, F)),
            "w_down": _w((lambda *s: _rng.normal(s) * 0.05)(F, D)),
        }
    _B_in = _B_setup()

    return {
        "A_x": _A_in["x"],
        "A_wqkv": _A_in["wqkv"],
        "A_w_phi": _A_in["w_phi"],
        "A_wo": _A_in["wo"],
        "B_x": _B_in["x"],
        "B_w_gate": _B_in["w_gate"],
        "B_w_up": _B_in["w_up"],
        "B_w_down": _B_in["w_down"],
    }

def reference(A_x, A_wqkv, A_w_phi, A_wo, B_x, B_w_gate, B_w_up, B_w_down):
    def _A_ref(x, wqkv, w_phi, wo):
        B, S, D = x.shape
        H = 32; Dh = D // H
        qkv = (lambda x, *d: x.transpose(*d))((x @ wqkv).reshape(B, S, 3, H, Dh), 2, 0, 3, 1, 4)
        q, k, v = qkv[0], qkv[1], qkv[2]
        pq = jnp.einsum("bhsd,hdf->bhsf", q, w_phi)
        pk = jnp.einsum("bhsd,hdf->bhsf", k, w_phi)
        phi_q = jnp.concatenate([_softmax(pq, axis=-1), _softmax(-pq, axis=-1)], axis=-1)
        phi_k = jnp.concatenate([_softmax(pk, axis=-1), _softmax(-pk, axis=-1)], axis=-1)
        kv = jnp.einsum("bhsf,bhsd->bhfd", phi_k, v)
        z  = jnp.einsum("bhsf->bhf", phi_k)
        num = jnp.einsum("bhqf,bhfd->bhqd", phi_q, kv)
        den = jnp.einsum("bhqf,bhf->bhq", phi_q, z)[..., None] + 1e-6
        o = num / den
        return (lambda x, *d: x.transpose(*d))(o, 0, 2, 1, 3).reshape(B, S, D) @ wo

    def _B_ref(x, w_gate, w_up, w_down):
        return (_gelu(x @ w_gate) * (x @ w_up)) @ w_down

    x = A_x
    h = x + _A_ref(_layernorm(x, axis=-1), A_wqkv, A_w_phi, A_wo)
    h2 = h + _B_ref(_layernorm(h, axis=-1), B_w_gate, B_w_up, B_w_down)
    return h2
```

```python
import numpy as np
import jax
import jax.numpy as jnp
from jax import lax
import jax.experimental.pallas as pl
import jax.experimental.pallas.tpu as pltpu

S, D, H, DH, F = 2048, 640, 32, 20, 1536
HG = 2
GW = HG * DH
NG = H // HG
NV = GW // 8
ND = D // 128
T = 512
NT = S // T
RB = 256
FC = 512
CG = 2
WR = 16
R0, RV, R1 = 160, 320, 160
WO = (0, 2, 5)
LOG2E = float(np.log2(np.e))

f32, bf16 = jnp.float32, jnp.bfloat16


def _fold_spans():
    n = max(((lo + 127) // GW + 1 - lo // GW) * GW for lo in range(0, D, 128))
    return [(lo, lo + 128, min(lo // GW * GW, D - n), min(lo // GW * GW, D - n) + n) for lo in range(0, D, 128)]


FOLDS = _fold_spans()


def _dot(a, b):
    return jnp.dot(a, b, preferred_element_type=f32)


def _dot_nt(a, b):
    return lax.dot_general(a, b, (((1,), (1,)), ((), ())), preferred_element_type=f32)


def _iota(shape, axis):
    return lax.broadcasted_iota(jnp.int32, shape, axis)


def _overlap_add(spans, parts):
    cuts = sorted({v for sp in spans for v in sp[2:]})
    segs = []
    for lo, hi in zip(cuts[:-1], cuts[1:]):
        terms = [p[lo - a:hi - a] for (_, _, a, b), p in zip(spans, parts) if a <= lo and hi <= b]
        segs.append(sum(terms[1:], terms[0]))
    return jnp.concatenate(segs, axis=0)


def _recip(x):
    r = pl.reciprocal(x, approx=True)
    return r * (2.0 - x * r)


def _ln(x):
    m = jnp.mean(x, axis=-1, keepdims=True)
    xc = x - m
    v = jnp.mean(xc * xc, axis=-1, keepdims=True)
    return xc * lax.rsqrt(v + 1e-5)


def _gelu(x):
    c = float(np.sqrt(2.0 / np.pi))
    hx = 0.5 * x
    return hx + hx * jnp.tanh(x * (c + (c * 0.044715) * (x * x)))


def _head_reduce(a, op):
    r = a[:, 0]
    for i in range(1, NV):
        r = op(r, a[:, i])
    for s in (4, 2):
        r = op(r, pltpu.roll(r, s, 1))
    return r[:, None]


def _features(p, g0):
    p4 = p[g0 * GW:(g0 + CG) * GW].reshape(CG, NV, 8, p.shape[-1])
    ep = jnp.exp2(p4 - _head_reduce(p4, jnp.maximum))
    en = jnp.exp2(_head_reduce(p4, jnp.minimum) - p4)
    sp, sn = _head_reduce(ep, jnp.add), _head_reduce(en, jnp.add)
    r = _recip(sp * sn)
    ph = jnp.concatenate([ep * (sn * r), en * (sp * r)], axis=1).reshape(-1, p.shape[-1])
    return [ph[2 * GW * k:2 * GW * (k + 1)].astype(bf16) for k in range(CG)]


def _lhs_terms(a):
    n = a.shape[0] // 2
    a11, a12, a21, a22 = a[:n, :256], a[:n, 256:], a[n:, :256], a[n:, 256:]
    return [t.astype(bf16) for t in (a11 + a22, a21 + a22, a11, a22, a11 + a12, a21 - a11, a12 - a22)]


def _store_rhs_sums(s_ref, block, w_ref, r0, c0):
    for r in range(0, 256, WR):
        b11, b12, b21, b22 = (w_ref[r0 + i + r:r0 + i + r + WR, c0 + j:c0 + j + 256].astype(f32)
                              for i in (0, 256) for j in (0, 256))
        for k, v in enumerate((b11 + b22, b12 - b22, b21 - b11, b11 + b12, b21 + b22)):
            s_ref[block, k, r:r + WR, :] = v.astype(bf16)


def _products(lhs, s_ref, block, w_ref, r0, c0):
    s = [s_ref[block, k] for k in range(5)]
    b11, b22 = (w_ref[r0 + i:r0 + i + 256, c0 + i:c0 + i + 256] for i in (0, 256))
    return [_dot(a, b) for a, b in zip(lhs, (s[0], b11, s[1], s[2], b22, s[3], s[4]))]


def _combine(m):
    top = jnp.concatenate([m[0] + m[3] - m[4] + m[6], m[2] + m[4]], axis=1)
    bot = jnp.concatenate([m[1] + m[3], m[0] - m[1] + m[2] + m[5]], axis=1)
    return jnp.concatenate([top, bot], axis=0)


def _kernel(x_hbm, wphi_hbm, wqkv_hbm, wo_hbm, wg_hbm, wu_hbm, wd_hbm, o_hbm,
            x_v, wphi_v, wk_v, wq_v, wv_v, wo_v, wg_v, wu_v, wd_v, out_v,
            wkT, wvT, wqT, xn_v, kvT, sums_v, sems):

    def rows_of(i, t):
        return pl.ds(i * t if isinstance(i, int) else pl.multiple_of(i * t, t), t)

    def x_piece(lo, hi):
        return x_hbm.at[0, pl.ds(lo, hi - lo)], x_v.at[pl.ds(lo, hi - lo)]

    def qkv_piece(k, dst):
        return wqkv_hbm.at[:, pl.ds(k * D, D)], dst

    stages = [
        [(wphi_hbm, wphi_v)],
        [qkv_piece(1, wk_v)],
        [x_piece(0, T // 2)],
        [x_piece(T // 2, T), qkv_piece(2, wv_v)],
        [x_piece(T, S)],
        [qkv_piece(0, wq_v), (wo_hbm, wo_v), (wg_hbm, wg_v), (wu_hbm, wu_v), (wd_hbm, wd_v)],
    ]

    def wait(k):
        for src, dst in stages[k]:
            pltpu.make_async_copy(src, dst, sems.at[k]).wait()

    def o_copy(r):
        return pltpu.make_async_copy(out_v.at[rows_of(r, RB)], o_hbm.at[0, rows_of(r, RB)], sems.at[len(stages)])

    for k, stage in enumerate(stages):
        for src, dst in stage:
            pltpu.make_async_copy(src, dst, sems.at[k]).start()

    nrow = FOLDS[0][3] - FOLDS[0][2]
    shp = (nrow // GW, NV, 8, DH)
    feat = _iota(shp, 1) * (8 // HG) + (_iota(shp, 2) >> 1)
    expand = (feat == _iota(shp, 3)).astype(f32).reshape(nrow, DH).astype(bf16)
    base = _iota((H, D), 1) - _iota((H, D), 0) * DH
    perm = jnp.concatenate([(base == d).astype(f32) for d in range(DH)], axis=0).astype(bf16)
    wait(0)
    y = jnp.concatenate([wphi_v[d].astype(f32) for d in range(DH)], axis=1).astype(bf16)
    y = _dot(y, perm).astype(bf16)
    y = _dot(expand, y)
    shp = (nrow // GW, NV, 8, 128)
    off = _iota(shp, 3) - (_iota(shp, 0) * HG + (_iota(shp, 2) & 1)) * DH
    maps = []
    for lo, hi, a, _ in FOLDS:
        m = jnp.where((off >= a - lo) & (off < a - lo + DH), y[:, lo:hi].reshape(shp), 0.0)
        maps.append(m.reshape(nrow, 128).astype(bf16))

    def fold(w_ref):
        parts = [_dot_nt(maps[j], w_ref[:, 128 * j:128 * (j + 1)]) for j in range(ND)]
        return (_overlap_add(FOLDS, parts) * LOG2E).astype(bf16)

    def norm(lo, n):
        xn = _ln(x_v[lo:lo + n, :].astype(f32)).astype(bf16)
        xn_v[lo:lo + n, :] = xn
        return xn

    def proj(w, i, lo=0, hi=D // 2):
        xn = xn_v[rows_of(i, T), :]
        return tuple(_dot_nt(w[r + lo:r + hi, :], xn) for r in (0, D // 2))

    def rows(*halves):
        return jnp.concatenate(halves[0::2] + halves[1::2], axis=0)

    acc = [None] * NG
    ones = jnp.ones((8, T), f32)

    def accumulate(pk, vt):
        for g0 in range(0, NG, CG):
            for k, ph in enumerate(_features(pk, g0)):
                g = g0 + k
                v1 = jnp.concatenate([vt[g * GW:(g + 1) * GW], ones], axis=0).astype(bf16)
                t = _dot_nt(v1, ph)
                acc[g] = t if acc[g] is None else acc[g] + t

    wait(1)
    wait(2)
    wkT[...] = fold(wk_v)
    xa = norm(0, T // 2)
    pa = _dot_nt(wkT[:R0, :], xa)
    wait(3)
    pa = jnp.concatenate([pa, _dot_nt(wkT[R0:, :], xa)], axis=0)
    xb = norm(T // 2, T // 2)
    wvT[...] = wv_v[...].T
    pk0 = jnp.concatenate([pa, _dot_nt(wkT[...], xb)], axis=1)
    vt0 = jnp.concatenate([_dot_nt(wvT[:RV, :], xa), _dot_nt(wvT[:RV, :], xb)], axis=1)
    wait(4)
    rest = jnp.concatenate([_dot_nt(wvT[RV:, :], xa), _dot_nt(wvT[RV:, :], xb)], axis=1)
    vt0 = jnp.concatenate([vt0, rest], axis=0)
    norm(T, T)
    head = proj(wkT, 1, 0, R1)
    accumulate(pk0, vt0)
    pk, vt = rows(*head, *proj(wkT, 1, R1)), rows(*proj(wvT, 1))
    for i in range(1, NT):
        if i + 1 < NT:
            norm((i + 1) * T, T)
        accumulate(pk, vt)
        if i + 1 < NT:
            pk, vt = rows(*proj(wkT, i + 1)), rows(*proj(wvT, i + 1))

    wait(5)
    wqT[...] = fold(wq_v)
    r = _iota((GW + 8, 2 * GW), 0)
    second = ((r >= DH) & (r < GW)) | (r >= GW + 4)
    keep = second == ((_iota((GW + 8, 2 * GW), 1) & 1) == 1)
    for g in range(NG):
        kvT[g] = jnp.where(keep, acc[g], 0.0).astype(bf16)
    nc = F // FC
    for c in range(nc):
        _store_rhs_sums(sums_v, c, wg_v, 0, c * FC)
    for c in range(nc):
        _store_rhs_sums(sums_v, nc + c, wu_v, 0, c * FC)
    for c in range(nc):
        _store_rhs_sums(sums_v, 2 * nc + c, wd_v, c * FC, 0)

    @pl.loop(0, NT)
    def _(i):
        nb = T // RB
        low = _iota((8, T), 0) < 4
        pq = rows(*proj(wqT, i))
        parts = []
        for g0 in range(0, NG, CG):
            for k, ph in enumerate(_features(pq, g0)):
                t = _dot(kvT[g0 + k], ph)
                r = _recip(t[GW:] + 1e-6)
                s = pltpu.roll(r, 4, 0)
                r0, r1 = jnp.where(low, r, s), jnp.where(low, s, r)
                parts.append(t[:GW] * jnp.concatenate([r0, r0, r, r1, r1], axis=0))
        hs = [x_v[rows_of(i * nb + b, RB), :].astype(f32) for b in range(nb)]
        for lo, hi in zip(WO[:-1], WO[1:]):
            o = jnp.concatenate(parts, axis=0)[128 * lo:128 * hi].T
            for b in range(nb):
                hs[b] = hs[b] + _dot(o[b * RB:(b + 1) * RB].astype(bf16), wo_v[128 * lo:128 * hi, :])

        state = []
        for h in hs:
            hn = _ln(h)
            state.append(dict(h=h, lhs=_lhs_terms(hn[:, :512]), last=hn[:, 512:].astype(bf16),
                              main=None, edge=h[:, 512:]))

        def hidden(b, c):
            st, res = state[b], []
            for n, w in enumerate((wg_v, wu_v)):
                edge = _dot(st["last"], w[512:, c * FC:(c + 1) * FC])
                res.append(_combine(_products(st["lhs"], sums_v, n * nc + c, w, 0, c * FC)) + edge)
            return _gelu(res[0]) * res[1]

        def down(b, c, act):
            st = state[b]
            m = _products(_lhs_terms(act), sums_v, 2 * nc + c, wd_v, c * FC, 0)
            st["edge"] = st["edge"] + _dot(act.astype(bf16), wd_v[c * FC:(c + 1) * FC, 512:])
            st["main"] = m if c == 0 else [p + q for p, q in zip(st["main"], m)]
            if c == nc - 1:
                y = jnp.concatenate([st["h"][:, :512] + _combine(st["main"]), st["edge"]], axis=1)
                out_v[rows_of(i * nb + b, RB), :] = y.astype(out_v.dtype)
                o_copy(i * nb + b).start()

        jobs = [(b, c) for b in range(nb) for c in range(nc)]
        act = hidden(*jobs[0])
        for k, job in enumerate(jobs):
            nxt = hidden(*jobs[k + 1]) if k + 1 < len(jobs) else None
            down(*job, act)
            act = nxt

    for b in range(S // RB):
        o_copy(b).wait()


@jax.jit
def pallas_sequential_preLN__linear_kernel_hedgehog__geglu_ffn__prompt_kernel(
    A_x: jax.Array,
    A_wqkv: jax.Array,
    A_w_phi: jax.Array,
    A_wo: jax.Array,
    B_x: jax.Array,
    B_w_gate: jax.Array,
    B_w_up: jax.Array,
    B_w_down: jax.Array,
):
    del B_x
    hbm = pl.BlockSpec(memory_space=pl.ANY)
    return pl.pallas_call(
        _kernel,
        in_specs=[hbm] * 7,
        out_specs=hbm,
        out_shape=jax.ShapeDtypeStruct((1, S, D), A_x.dtype),
        scratch_shapes=[
            pltpu.VMEM((S, D), bf16), pltpu.VMEM((DH, DH, H), bf16),
            pltpu.VMEM((D, D), bf16), pltpu.VMEM((D, D), bf16), pltpu.VMEM((D, D), bf16),
            pltpu.VMEM((D, D), bf16),
            pltpu.VMEM((D, F), bf16), pltpu.VMEM((D, F), bf16), pltpu.VMEM((F, D), bf16),
            pltpu.VMEM((S, D), A_x.dtype),
            pltpu.VMEM((D, D), bf16), pltpu.VMEM((D, D), bf16), pltpu.VMEM((D, D), bf16),
            pltpu.VMEM((S, D), bf16),
            pltpu.VMEM((NG, GW + 8, 2 * GW), bf16),
            pltpu.VMEM((3 * F // FC, 5, 256, 256), bf16),
            pltpu.SemaphoreType.DMA((7,)),
        ],
        compiler_params=pltpu.CompilerParams(vmem_limit_bytes=100 * 1024 * 1024),
    )(A_x, jnp.transpose(A_w_phi, (1, 2, 0)), A_wqkv, A_wo, B_w_gate, B_w_up, B_w_down)
```

```python
import numpy as np
import jax
import jax.numpy as jnp
from jax import lax
import jax.experimental.pallas as pl
import jax.experimental.pallas.tpu as pltpu

S, D, H, DH, F = 2048, 640, 32, 20, 1536
HG = 2
GW = HG * DH
NG = H // HG
NV = GW // 8
ND = D // 128
T = 512
NT = S // T
RB = 256
FC = 512
CG = 2
RS = 160
RW = 112
WO = (0, 2, 5)
LOG2E = float(np.log2(np.e))

f32, bf16 = jnp.float32, jnp.bfloat16


def _fold_spans():
    n = max(((lo + 127) // GW + 1 - lo // GW) * GW for lo in range(0, D, 128))
    return [(lo, lo + 128, min(lo // GW * GW, D - n), min(lo // GW * GW, D - n) + n) for lo in range(0, D, 128)]


FOLDS = _fold_spans()


def _dot(a, b):
    return jnp.dot(a, b, preferred_element_type=f32)


def _dot_nt(a, b):
    return lax.dot_general(a, b, (((1,), (1,)), ((), ())), preferred_element_type=f32)


def _iota(shape, axis):
    return lax.broadcasted_iota(jnp.int32, shape, axis)


def _overlap_add(spans, parts):
    cuts = sorted({v for sp in spans for v in sp[2:]})
    segs = []
    for lo, hi in zip(cuts[:-1], cuts[1:]):
        terms = [p[lo - a:hi - a] for (_, _, a, b), p in zip(spans, parts) if a <= lo and hi <= b]
        segs.append(sum(terms[1:], terms[0]))
    return jnp.concatenate(segs, axis=0)


def _recip(x):
    r = pl.reciprocal(x, approx=True)
    return r * (2.0 - x * r)


def _ln(x):
    m = jnp.mean(x, axis=-1, keepdims=True)
    xc = x - m
    v = jnp.mean(xc * xc, axis=-1, keepdims=True)
    return xc * lax.rsqrt(v + 1e-5)


def _gelu(x):
    c = float(np.sqrt(2.0 / np.pi))
    hx = 0.5 * x
    return hx + hx * jnp.tanh(x * (c + (c * 0.044715) * (x * x)))


def _head_reduce(a, op):
    r = a[:, 0]
    for i in range(1, NV):
        r = op(r, a[:, i])
    for s in (4, 2):
        r = op(r, pltpu.roll(r, s, 1))
    return r[:, None]


def _features(p, g0):
    p4 = p[g0 * GW:(g0 + CG) * GW].reshape(CG, NV, 8, p.shape[-1])
    ep = jnp.exp2(p4 - _head_reduce(p4, jnp.maximum))
    en = jnp.exp2(_head_reduce(p4, jnp.minimum) - p4)
    sp, sn = _head_reduce(ep, jnp.add), _head_reduce(en, jnp.add)
    r = _recip(sp * sn)
    ph = jnp.concatenate([ep * (sn * r), en * (sp * r)], axis=1).reshape(-1, p.shape[-1])
    return [ph[2 * GW * k:2 * GW * (k + 1)].astype(bf16) for k in range(CG)]


def _lhs_terms(a):
    n = a.shape[0] // 2
    a11, a12, a21, a22 = a[:n, :256], a[:n, 256:], a[n:, :256], a[n:, 256:]
    return [t.astype(bf16) for t in (a11 + a22, a21 + a22, a11, a22, a11 + a12, a21 - a11, a12 - a22)]


def _store_rhs_sums(s_ref, block, w_ref, r0, c0, zero):
    for r in range(0, 256, 8):
        b11, b12, b21, b22 = (w_ref[r0 + i + r:r0 + i + r + 8, c0 + j:c0 + j + 256].astype(f32)
                              for i in (0, 256) for j in (0, 256))
        zero = jnp.tanh(jnp.tanh(zero))
        z = jnp.tile(zero, (1, 2))
        b11, b22 = b11 + z, b22 + z
        for k, v in enumerate((b11 + b22, b12 - b22, b21 - b11, b11 + b12, b21 + b22)):
            s_ref[block, k, r:r + 8, :] = v.astype(bf16)
    return zero


def _products(lhs, s_ref, block, w_ref, r0, c0):
    s = [s_ref[block, k] for k in range(5)]
    b11, b22 = (w_ref[r0 + i:r0 + i + 256, c0 + i:c0 + i + 256] for i in (0, 256))
    rhs = (s[0], b11, s[1], s[2], b22, s[3], s[4])
    m = {k: _dot(lhs[k], rhs[k]) for k in (2, 4, 6, 0, 3, 1, 5)}
    return [m[k] for k in range(7)]


def _combine(m):
    top = jnp.concatenate([m[0] + m[3] - m[4] + m[6], m[2] + m[4]], axis=1)
    bot = jnp.concatenate([m[1] + m[3], m[0] - m[1] + m[2] + m[5]], axis=1)
    return jnp.concatenate([top, bot], axis=0)


def _kernel(x_hbm, wphi_hbm, wqkv_hbm, wo_hbm, wg_hbm, wu_hbm, wd_hbm, o_hbm,
            x_v, wphi_v, wk_v, wq_v, wv_v, wo_v, wg_v, wu_v, wd_v, out_v,
            wkT, wvT, wqT, xn_v, kvT, sums_v, sems):

    def rows_of(i, t):
        return pl.ds(i * t if isinstance(i, int) else pl.multiple_of(i * t, t), t)

    def x_piece(lo, hi):
        return x_hbm.at[0, pl.ds(lo, hi - lo)], x_v.at[pl.ds(lo, hi - lo)]

    def qkv_piece(k, dst):
        return wqkv_hbm.at[:, pl.ds(k * D, D)], dst

    stages = [
        [(wphi_hbm, wphi_v)],
        [x_piece(0, T // 2)],
        [qkv_piece(1, wk_v)],
        [qkv_piece(2, wv_v)],
        [x_piece(T // 2, T)],
        [x_piece(T, S)],
        [qkv_piece(0, wq_v), (wo_hbm, wo_v), (wg_hbm, wg_v), (wu_hbm, wu_v), (wd_hbm, wd_v)],
    ]

    def wait(k):
        for src, dst in stages[k]:
            pltpu.make_async_copy(src, dst, sems.at[k]).wait()

    def o_copy(r):
        return pltpu.make_async_copy(out_v.at[rows_of(r, RB)], o_hbm.at[0, rows_of(r, RB)], sems.at[len(stages)])

    for k, stage in enumerate(stages):
        for src, dst in stage:
            pltpu.make_async_copy(src, dst, sems.at[k]).start()

    nrow = FOLDS[0][3] - FOLDS[0][2]
    shp = (nrow // GW, NV, 8, DH)
    feat = _iota(shp, 1) * (8 // HG) + (_iota(shp, 2) >> 1)
    expand = (feat == _iota(shp, 3)).astype(f32).reshape(nrow, DH).astype(bf16)
    base = _iota((H, D), 1) - _iota((H, D), 0) * DH
    perm = jnp.concatenate([(base == d).astype(f32) for d in range(DH)], axis=0).astype(bf16)
    wait(0)
    y = jnp.concatenate([wphi_v[d].astype(f32) for d in range(DH)], axis=1).astype(bf16)
    y = _dot(y, perm).astype(bf16)
    y = _dot(expand, y)
    shp = (nrow // GW, NV, 8, 128)
    off = _iota(shp, 3) - (_iota(shp, 0) * HG + (_iota(shp, 2) & 1)) * DH
    maps = []
    for lo, hi, a, _ in FOLDS:
        m = jnp.where((off >= a - lo) & (off < a - lo + DH), y[:, lo:hi].reshape(shp), 0.0)
        maps.append(m.reshape(nrow, 128).astype(bf16))

    def fold(w_ref):
        parts = [_dot_nt(maps[j], w_ref[:, 128 * j:128 * (j + 1)]) for j in range(ND)]
        return (_overlap_add(FOLDS, parts) * LOG2E).astype(bf16)

    def norm(lo, n):
        xn = _ln(x_v[lo:lo + n, :].astype(f32)).astype(bf16)
        xn_v[lo:lo + n, :] = xn
        return xn

    def proj(w, i, lo=0, hi=D // 2):
        xn = xn_v[rows_of(i, T), :]
        return tuple(_dot_nt(w[r + lo:r + hi, :], xn) for r in (0, D // 2))

    def rows(*halves):
        return jnp.concatenate(halves[0::2] + halves[1::2], axis=0)

    acc = [None] * NG
    ones = jnp.ones((8, T), f32)

    def accumulate(pk, vt):
        for g0 in range(0, NG, CG):
            for k, ph in enumerate(_features(pk, g0)):
                g = g0 + k
                v1 = jnp.concatenate([vt[g * GW:(g + 1) * GW], ones], axis=0).astype(bf16)
                t = _dot_nt(v1, ph)
                acc[g] = t if acc[g] is None else acc[g] + t

    wait(1)
    xa = norm(0, T // 2)
    wait(2)
    wkT[...] = fold(wk_v)
    pa = _dot_nt(wkT[:RS, :], xa)
    wait(3)
    pa = jnp.concatenate([pa, _dot_nt(wkT[RS:, :], xa)], axis=0)
    wvT[...] = wv_v[...].T
    va = _dot_nt(wvT[:RS, :], xa)
    wait(4)
    va = jnp.concatenate([va, _dot_nt(wvT[RS:, :], xa)], axis=0)
    xb = norm(T // 2, T // 2)
    pk0 = jnp.concatenate([pa, _dot_nt(wkT[...], xb)], axis=1)
    vb = _dot_nt(wvT[:RS, :], xb)
    wait(5)
    vb = jnp.concatenate([vb, _dot_nt(wvT[RS:, :], xb)], axis=0)
    vt0 = jnp.concatenate([va, vb], axis=1)
    norm(T, T)
    head = proj(wkT, 1, 0, RS)
    accumulate(pk0, vt0)
    pk, vt = rows(*head, *proj(wkT, 1, RS)), rows(*proj(wvT, 1))
    for i in range(1, NT):
        if i + 1 < NT:
            norm((i + 1) * T, T)
        accumulate(pk, vt)
        if i + 2 < NT:
            pk, vt = rows(*proj(wkT, i + 1)), rows(*proj(wvT, i + 1))
        elif i + 1 < NT:
            head = proj(wkT, i + 1, 0, RW)
            wait(6)
            pk, vt = rows(*head, *proj(wkT, i + 1, RW)), rows(*proj(wvT, i + 1))

    wqT[...] = fold(wq_v)
    r = _iota((GW + 8, 2 * GW), 0)
    second = ((r >= DH) & (r < GW)) | (r >= GW + 4)
    keep = second == ((_iota((GW + 8, 2 * GW), 1) & 1) == 1)
    for g in range(NG):
        kvT[g] = jnp.where(keep, acc[g], 0.0).astype(bf16)
    nc = F // FC
    zero = jnp.minimum(jnp.maximum(head[0][:8, :128], 0.0), 0.0)
    blocks = ([(wg_v, 0, c * FC) for c in range(nc)] + [(wu_v, 0, c * FC) for c in range(nc)]
              + [(wd_v, c * FC, 0) for c in range(nc)])
    for k, block in enumerate(blocks):
        zero = _store_rhs_sums(sums_v, k, *block, zero)

    @pl.loop(0, NT)
    def _(i):
        nb = T // RB
        low = _iota((8, T), 0) < 4
        pq = rows(*proj(wqT, i))
        parts = []
        for g0 in range(0, NG, CG):
            for k, ph in enumerate(_features(pq, g0)):
                t = _dot(kvT[g0 + k], ph)
                r = _recip(t[GW:] + 1e-6)
                s = pltpu.roll(r, 4, 0)
                r0, r1 = jnp.where(low, r, s), jnp.where(low, s, r)
                parts.append(t[:GW] * jnp.concatenate([r0, r0, r, r1, r1], axis=0))
        hs = [x_v[rows_of(i * nb + b, RB), :].astype(f32) for b in range(nb)]
        for lo, hi in zip(WO[:-1], WO[1:]):
            o = jnp.concatenate(parts, axis=0)[128 * lo:128 * hi].T
            for b in range(nb):
                hs[b] = hs[b] + _dot(o[b * RB:(b + 1) * RB].astype(bf16), wo_v[128 * lo:128 * hi, :])

        state = []
        for h in hs:
            hn = _ln(h)
            state.append(dict(h=h, lhs=_lhs_terms(hn[:, :512]), last=hn[:, 512:].astype(bf16),
                              main=None, edge=h[:, 512:]))

        def hidden(b, c):
            st, res = state[b], []
            for n, w in enumerate((wg_v, wu_v)):
                edge = _dot(st["last"], w[512:, c * FC:(c + 1) * FC])
                res.append(_combine(_products(st["lhs"], sums_v, n * nc + c, w, 0, c * FC)) + edge)
            return _gelu(res[0]) * res[1]

        def down(b, c, act):
            st = state[b]
            m = _products(_lhs_terms(act), sums_v, 2 * nc + c, wd_v, c * FC, 0)
            st["edge"] = st["edge"] + _dot(act.astype(bf16), wd_v[c * FC:(c + 1) * FC, 512:])
            st["main"] = m if c == 0 else [p + q for p, q in zip(st["main"], m)]
            if c == nc - 1:
                y = jnp.concatenate([st["h"][:, :512] + _combine(st["main"]), st["edge"]], axis=1)
                out_v[rows_of(i * nb + b, RB), :] = y.astype(out_v.dtype)
                o_copy(i * nb + b).start()

        jobs = [(b, c) for b in range(nb) for c in range(nc)]
        act = hidden(*jobs[0])
        for k, job in enumerate(jobs):
            nxt = hidden(*jobs[k + 1]) if k + 1 < len(jobs) else None
            down(*job, act)
            act = nxt

    for b in range(S // RB):
        o_copy(b).wait()


@jax.jit
def pallas_sequential_preLN__linear_kernel_hedgehog__geglu_ffn__prompt_kernel(
    A_x: jax.Array,
    A_wqkv: jax.Array,
    A_w_phi: jax.Array,
    A_wo: jax.Array,
    B_x: jax.Array,
    B_w_gate: jax.Array,
    B_w_up: jax.Array,
    B_w_down: jax.Array,
):
    del B_x
    hbm = pl.BlockSpec(memory_space=pl.ANY)
    return pl.pallas_call(
        _kernel,
        in_specs=[hbm] * 7,
        out_specs=hbm,
        out_shape=jax.ShapeDtypeStruct((1, S, D), A_x.dtype),
        scratch_shapes=[
            pltpu.VMEM((S, D), bf16), pltpu.VMEM((DH, DH, H), bf16),
            pltpu.VMEM((D, D), bf16), pltpu.VMEM((D, D), bf16), pltpu.VMEM((D, D), bf16),
            pltpu.VMEM((D, D), bf16),
            pltpu.VMEM((D, F), bf16), pltpu.VMEM((D, F), bf16), pltpu.VMEM((F, D), bf16),
            pltpu.VMEM((S, D), A_x.dtype),
            pltpu.VMEM((D, D), bf16), pltpu.VMEM((D, D), bf16), pltpu.VMEM((D, D), bf16),
            pltpu.VMEM((S, D), bf16),
            pltpu.VMEM((NG, GW + 8, 2 * GW), bf16),
            pltpu.VMEM((3 * F // FC, 5, 256, 256), bf16),
            pltpu.SemaphoreType.DMA((8,)),
        ],
        compiler_params=pltpu.CompilerParams(vmem_limit_bytes=100 * 1024 * 1024),
    )(A_x, jnp.transpose(A_w_phi, (1, 2, 0)), A_wqkv, A_wo, B_w_gate, B_w_up, B_w_down)
```
